```python
import jax
import jax.numpy as jnp

def _softmax(x, axis=-1):
    return jax.nn.softmax(x, axis=axis)

def _gelu(x):
    return jax.nn.gelu(x, approximate=True)

def _silu(x):
    return jax.nn.silu(x)

def _sigmoid(x):
    return jax.nn.sigmoid(x)

def _layernorm(x, axis=-1, eps=1e-05):
    m = jnp.mean(x, axis=axis, keepdims=True)
    v = jnp.var(x, axis=axis, keepdims=True)
    return (x - m) / jnp.sqrt(v + eps)

def _scatter_add(tgt, idx, src, axis=0):
    return tgt.at[idx].add(src)

def _segment_sum(src, seg, n):
    return jax.ops.segment_sum(src, seg, n)

class _Rng:

    def __init__(self, key):
        self._k = key

    def _next(self):
        self._k, sub = jax.random.split(self._k)
        return sub

    def normal(self, shape):
        return jax.random.normal(self._next(), shape, dtype=jnp.bfloat16)

    def randint(self, lo, hi, shape):
        return jax.random.randint(self._next(), shape, lo, hi, dtype=jnp.int32)

    def uniform(self, shape, lo=0.0, hi=1.0):
        return jax.random.uniform(self._next(), shape, jnp.bfloat16, lo, hi)

    def permutation(self, n):
        return jax.random.permutation(self._next(), n)
kernel_name = 'adaLN_cond__sliding_block_cached__glu_gated_swiglu__decode'

def setup_inputs():
    _rng = _Rng(jax.random.key(int.from_bytes(__import__("os").urandom(4), "little")))
    _w = lambda a: (lambda t: t.astype(jnp.bfloat16) if jnp.issubdtype(t.dtype, jnp.floating) else t)(jnp.asarray(a))

    def _A_setup():
        B, Sq, D = (2, 1, 512)
        Hq, Hkv, Sk, Dh = (32, 32, 16384, 128)
        assert Hq % Hkv == 0, (Hq, Hkv)
        return {'x': _w((lambda *s: _rng.normal(s) * 0.05)(B, Sq, D)), 'k_cache': _w((lambda *s: _rng.normal(s) * 0.05)(B, Hkv, Sk, Dh)), 'v_cache': _w((lambda *s: _rng.normal(s) * 0.05)(B, Hkv, Sk, Dh)), 'wq': _w((lambda *s: _rng.normal(s) * 0.05)(D, Hq * Dh) * D ** (-0.5)), 'wo': _w((lambda *s: _rng.normal(s) * 0.05)(Hq * Dh, D) * (Hq * Dh) ** (-0.5))}
    _A_in = _A_setup()

    def _B_setup():
        B, S, D, F = (2, 1, 512, 1376)
        return {'x': _w((lambda *s: _rng.normal(s) * 0.05)(B, S, D)), 'w1': _w((lambda *s: _rng.normal(s) * 0.05)(D, F) * (2.0 / D) ** 0.5), 'w3': _w((lambda *s: _rng.normal(s) * 0.05)(D, F) * (2.0 / D) ** 0.5), 'w2': _w((lambda *s: _rng.normal(s) * 0.05)(F, D) * (2.0 / F) ** 0.5)}
    _B_in = _B_setup()
    return {'A_x': _A_in['x'], 'A_k_cache': _A_in['k_cache'], 'A_v_cache': _A_in['v_cache'], 'A_wq': _A_in['wq'], 'A_wo': _A_in['wo'], 'B_x': _B_in['x'], 'B_w1': _B_in['w1'], 'B_w3': _B_in['w3'], 'B_w2': _B_in['w2'], 'c': _w((lambda *s: _rng.normal(s) * 0.05)(2, 512)), 'w_mod': _w((lambda *s: _rng.normal(s) * 0.05)(512, 6 * 512) * 512 ** (-0.5))}

def reference(A_x, A_k_cache, A_v_cache, A_wq, A_wo, B_x, B_w1, B_w3, B_w2, c, w_mod):

    def _A_ref(x, k_cache, v_cache, wq, wo):
        B, Sq, D = x.shape
        Hq, Dh = (32, 128)
        Hkv, Sk = (k_cache.shape[1], k_cache.shape[2])
        W = min(4096, max(256, Sk // 4))
        rep = Hq // Hkv
        q = (lambda x, *d: x.transpose(*d))((x @ wq).reshape(B, Sq, Hq, Dh), 0, 2, 1, 3)
        k = jnp.repeat(k_cache[:, :, Sk - W:, :], rep, axis=1)
        v = jnp.repeat(v_cache[:, :, Sk - W:, :], rep, axis=1)
        scores = jnp.einsum('bhqd,bhkd->bhqk', q, k) * Dh ** (-0.5)
        p = _softmax(scores, axis=-1)
        o = jnp.einsum('bhqk,bhkd->bhqd', p, v)
        return (lambda x, *d: x.transpose(*d))(o, 0, 2, 1, 3).reshape(B, Sq, Hq * Dh) @ wo

    def _B_ref(x, w1, w3, w2):
        gate = jnp.einsum('bsd,df->bsf', x, w1)
        up = jnp.einsum('bsd,df->bsf', x, w3)
        h = _silu(gate) * up
        out = jnp.einsum('bsf,fd->bsd', h, w2)
        return out
    x = A_x
    mod = (_silu(c) @ w_mod).reshape(c.shape[0], 6, 1, -1)
    sa, ca, ga, sb, cb, gb = (mod[:, 0].copy(), mod[:, 1].copy(), mod[:, 2].copy(), mod[:, 3].copy(), mod[:, 4].copy(), mod[:, 5].copy())
    h = _layernorm(x, axis=-1) * (1 + ca) + sa
    x = x + ga * _A_ref(h, A_k_cache, A_v_cache, A_wq, A_wo)
    h = _layernorm(x, axis=-1) * (1 + cb) + sb
    x = x + gb * _B_ref(h, B_w1, B_w3, B_w2)
    return x
```

```python
import jax
import jax.numpy as jnp
from jax import lax
import jax.experimental.pallas as pl
import jax.experimental.pallas.tpu as pltpu

F32 = jnp.float32
BF16 = jnp.bfloat16
NT = (((1,), (1,)), ((), ()))

def make(R=8, LA=7, fchunks=(384,384,384,128,96), fdesc=(64,256), pre=80, pi=8, ti=8, nosem=True):
    B, H, SK, DH, D, F = 2, 32, 16384, 128, 512, 1376
    W = min(4096, max(256, SK // 4))
    HG, TK, DR = 8, 128, 16
    UPG = W // TK
    NG = B * H // HG
    NU = NG * UPG
    scale = DH ** -0.5
    assert sum(fchunks) == F
    NC = len(fchunks)
    foff = [sum(fchunks[:i]) for i in range(NC)]
    S_X, S_C, S_M1, S_M2, S_WO, S_Q = 0, 1, 2, 3, 4, 5
    S_13 = S_Q + 4
    S_2 = S_13 + NC
    NWS = S_2 + NC

    def kernel(x_hbm, k_hbm, v_hbm, wq_hbm, wo_hbm, w1_hbm, w3_hbm, w2_hbm, c_hbm, wm_hbm, o_ref,
               kv, wq, wo, w1, w3, w2, wm, xc, sc_s, h1_s, q_s, o_s, mod_s, at_s, ksem, wsem):
        shr = lambda a, n: a >> n

        def kv_descs(u, s):
            g = shr(u, 5)
            r0 = (u & (UPG - 1)) * TK + (SK - W)
            b = g & 1
            h = shr(g, 1) * HG
            out = []
            for t in range(TK // DR):
                for j, src in enumerate((k_hbm, v_hbm)):
                    out.append(pltpu.make_async_copy(
                        src.at[b, pl.ds(h, HG), pl.ds(mo(r0 + t * DR, DR), DR)],
                        kv.at[s, j, :, pl.ds(t * DR, DR)], ksem.at[s]))
            return out

        def mo(v, m):
            return v if isinstance(v, int) else pl.multiple_of(v, m)

        def kv_wait(s):
            pltpu.make_async_copy(kv.at[s], kv.at[s], ksem.at[s]).wait()

        def wd(src, dst, si, r, c):
            r = mo(r, 8); c = mo(c, 512)
            return pltpu.make_async_copy(src.at[:, pl.ds(r, 8), pl.ds(c, 512)],
                                         dst.at[:, pl.ds(r, 8), pl.ds(c, 512)], wsem.at[si])

        def w_wait(dst, si, c0, nc):
            d = dst.at[:, :, pl.ds(mo(c0, 512), nc)]
            pltpu.make_async_copy(d, d, wsem.at[si]).wait()

        def fd(src, dst, si, r0, nr):
            br, bc = fdesc
            out = []
            r = 0
            while r < nr:
                if nr - r >= br:
                    for c in range(0, D, bc):
                        out.append((r, br, c, bc))
                    r += br
                else:
                    out.append((r, 32, 0, D))
                    r += 32
            return [pltpu.make_async_copy(src.at[pl.ds(r0 + r, n), pl.ds(c, w)],
                                          dst.at[pl.ds(r0 + r, n), pl.ds(c, w)], wsem.at[si])
                    for r, n, c, w in out]

        def f_wait(dst, si, r0, nr):
            d = dst.at[pl.ds(r0, nr)]
            pltpu.make_async_copy(d, d, wsem.at[si]).wait()

        def start_all(ds):
            for i, d in enumerate(ds):
                d.start(priority=i % 2)

        pending = []
        def issue(n):
            start_all(pending[:n])
            del pending[:n]

        def ln(x):
            m = jnp.mean(x, axis=-1, keepdims=True)
            xm = x - m
            v = jnp.mean(xm * xm, axis=-1, keepdims=True)
            return xm / jnp.sqrt(v + 1e-5)

        def rep(a):
            n = a.shape[1]
            return jnp.concatenate([jnp.broadcast_to(a[0:1], (8, n)), jnp.broadcast_to(a[1:2], (8, n))], axis=0)

        def mm4(lhs, w, c0, nc):
            acc = None
            for k in range(4):
                r = jnp.dot(lhs[:, k * 128:(k + 1) * 128], w[k, :, pl.ds(c0, nc)], preferred_element_type=F32)
                acc = r if acc is None else acc + r
            return acc

        row = lax.broadcasted_iota(jnp.int32, (HG, DH), 0)
        row16 = lax.broadcasted_iota(jnp.int32, (16, DH), 0) & 7

        def q_part(g, j, first):
            qq = mm4(h1_s[...], wq, mo(g * 1024 + j * 256, 256), 256)
            a, b = qq[:, :DH], qq[:, DH:]
            new = jnp.where(row16 == 2 * j, a, b)
            if first:
                q_s[g] = new
            else:
                q_s[g] = jnp.where(shr(row16, 1) == j, new, q_s[g])

        cx = pltpu.make_async_copy(x_hbm, xc.at[0], wsem.at[S_X])
        cc = pltpu.make_async_copy(c_hbm, xc.at[1], wsem.at[S_C])
        pending += [cc, cx]
        for i in range(16):
            pending += [wd(wm_hbm, wm, S_M1, i * 8, 0), wd(wm_hbm, wm, S_M1, i * 8, 512)]
        for i in range(16):
            pending += [wd(wq_hbm, wq, S_Q, i * 8, 0), wd(wq_hbm, wq, S_Q, i * 8, 512)]
        for u in range(LA):
            pending += kv_descs(u, u)
        issue(pre)
        cc.wait(); cx.wait()
        cv = xc[1].astype(F32)
        sc_s[...] = rep(cv * jax.nn.sigmoid(cv)).astype(BF16)
        x0 = rep(xc[0].astype(F32))
        lx = ln(x0)
        at_s[...] = jnp.zeros(at_s.shape, F32)
        w_wait(wm, S_M1, 0, 2 * D)
        parts = []
        for j in range(4):
            parts.append(mm4(sc_s[...], wm, j * 256, 256))
            issue(pi)
        sa = jnp.concatenate(parts[0:2], axis=1)
        ca = jnp.concatenate(parts[2:4], axis=1)
        h1_s[...] = (lx * (1.0 + ca) + sa).astype(BF16)
        w_wait(wq, S_Q, 0, 1024)
        for j in range(4):
            q_part(0, j, j == 0)
            issue(pi)
        issue(len(pending))

        def scores(u):
            s = u & (R - 1)
            g = shr(u, 5)
            q = q_s[shr(g, 1), pl.ds(mo((g & 1) * 8, 8), 8), :].astype(BF16)
            acc = None
            for h in range(HG):
                r = lax.dot_general(q, kv[s, 0, h], NT, preferred_element_type=F32)
                acc = r if acc is None else jnp.where(row == h, r, acc)
            return acc * scale

        def pv(u, s_, carry):
            m, l, acc = carry
            s = u & (R - 1)
            first = (u & (UPG - 1)) == 0
            m = jnp.where(first, -jnp.inf, m)
            l = jnp.where(first, 0.0, l)
            acc = jnp.where(first, 0.0, acc)
            m_new = jnp.maximum(m, jnp.max(s_, axis=-1, keepdims=True))
            alpha = jnp.exp(m - m_new)
            p = jnp.exp(s_ - m_new)
            l = alpha * l + p
            pb = p.astype(BF16)
            o = None
            for h in range(HG):
                r = jnp.dot(pb, kv[s, 1, h], preferred_element_type=F32)
                o = r if o is None else jnp.where(row == h, r, o)
            acc = alpha * acc + o
            return m_new, l, acc

        def finish(u, carry):
            m, l, acc = carry
            g = shr(u, 5)
            o_s[shr(g, 1), pl.ds(mo((g & 1) * 8, 8), 8), :] = acc / jnp.sum(l, axis=-1, keepdims=True)

        def wo_part(g, j):
            ob = o_s[g]
            acc = at_s[...]
            for e in range(2):
                h = 2 * j + e
                lhs = jnp.where(row16 == h, ob, 0.0).astype(BF16)
                acc = acc + jnp.dot(lhs, wo[g, pl.ds(mo(h * DH, DH), DH), :], preferred_element_type=F32)
            at_s[...] = acc

        def step(u, carry, descs, extra=None, last=False):
            s_, st = carry
            if not last:
                kv_wait((u + 1) & (R - 1))
            start_all(descs)
            if extra is not None:
                extra()
            s_next = s_ if last else scores(u + 1)
            st = pv(u, s_, st)
            if isinstance(u, int):
                if u % UPG == UPG - 1:
                    finish(u, st)
            else:
                pl.when((u & (UPG - 1)) == UPG - 1)(lambda: finish(u, st))
            return s_next, st

        U_Q, U_M, U_O = 48, 80, 144
        def sprinkle(u):
            @pl.when(u < U_Q)
            def _():
                g = shr(u, 4) + 1
                r = (u & 15) * 8
                start_all([wd(wq_hbm, wq, S_Q + g, r, g * 1024), wd(wq_hbm, wq, S_Q + g, r, g * 1024 + 512)])
            @pl.when((u >= U_Q) & (u < U_M))
            def _():
                i = u - U_Q
                r = (i & 15) * 8
                c = 2 * D + shr(i, 4) * 1024
                start_all([wd(wm_hbm, wm, S_M2, r, c), wd(wm_hbm, wm, S_M2, r, c + 512)])
            @pl.when((u >= U_M) & (u < U_O))
            def _():
                i = u - U_M
                start_all([wd(wo_hbm, wo, S_WO, i * 8, 0), wd(wo_hbm, wo, S_WO, 512 + i * 8, 0)])

        def extras(u):
            sprinkle(u)
            v = u & 63
            g = shr(u, 6)
            @pl.when((v == 56) & (g < 3))
            def _():
                w_wait(wq, S_Q + g + 1, (g + 1) * 1024, 1024)
                q_part(g + 1, 0, True)
            @pl.when((v > 56) & (v < 60) & (g < 3))
            def _():
                q_part(g + 1, v - 56, False)
            @pl.when(u == 96)
            def _():
                w_wait(wm, S_M2, 2 * D, 4 * D)
            @pl.when((u >= 96) & (u < 104))
            def _():
                c = mo((u - 96) * 256, 256)
                mod_s[:, pl.ds(c, 256)] = mm4(sc_s[...], wm, mo(2 * D + (u - 96) * 256, 256), 256)
            @pl.when(u == 160)
            def _():
                w_wait(wo, S_WO, 0, D)
            @pl.when(((u >= 160) & (u < 168)) | ((u >= 200) & (u < 204)))
            def _():
                i = jnp.where(u < 168, u - 160, u - 192)
                wo_part(shr(i, 2), i & 3)

        kv_wait(0)
        z = jnp.zeros((HG, DH), F32)
        carry = (scores(0), (jnp.full((HG, 1), -jnp.inf, F32), z, z))

        def body(u, carry):
            un = u + LA
            return step(u, carry, kv_descs(un, un & (R - 1)), lambda: extras(u))
        carry = lax.fori_loop(0, NU - LA, body, carry)

        for i in range(NC):
            a = fd(w1_hbm, w1, S_13 + i, foff[i], fchunks[i])
            b = fd(w3_hbm, w3, S_13 + i, foff[i], fchunks[i])
            for x, y in zip(a, b):
                pending += [x, y]
        n13 = len(pending)
        for i in range(NC):
            pending += fd(w2_hbm, w2, S_2 + i, foff[i], fchunks[i])

        for u in range(NU - LA, NU):
            ds = pending[:16]
            del pending[:16]
            carry = step(u, carry, ds, last=(u == NU - 1))
        for j in range(4):
            wo_part(3, j)
            issue(ti)
        issue(len(pending))
        at = at_s[...]
        attn = jnp.concatenate(
            [jnp.broadcast_to(jnp.sum(at[b * 8:(b + 1) * 8], axis=0, keepdims=True), (8, D)) for b in range(B)], axis=0)
        x1 = rep(xc[0].astype(F32)) + mod_s[:, 0:D] * attn
        h2 = (ln(x1) * (1.0 + mod_s[:, 2 * D:3 * D]) + mod_s[:, D:2 * D]).astype(BF16)
        hs = []
        for i in range(NC):
            r0, n = foff[i], fchunks[i]
            f_wait(w1, S_13 + i, r0, n)
            f_wait(w3, S_13 + i, r0, n)
            gate = lax.dot_general(h2, w1[r0:r0 + n, :], NT, preferred_element_type=F32)
            up = lax.dot_general(h2, w3[r0:r0 + n, :], NT, preferred_element_type=F32)
            hs.append((gate * jax.nn.sigmoid(gate) * up).astype(BF16))
        ff = None
        for i in range(NC):
            r0, n = foff[i], fchunks[i]
            f_wait(w2, S_2 + i, r0, n)
            r = jnp.dot(hs[i], w2[r0:r0 + n, :], preferred_element_type=F32)
            ff = r if ff is None else ff + r
        y = x1 + mod_s[:, 3 * D:4 * D] * ff
        o_ref[...] = jnp.concatenate([y[0:1], y[8:9]], axis=0).astype(o_ref.dtype)

    def fn(A_x, A_k_cache, A_v_cache, A_wq, A_wo, B_x, B_w1, B_w3, B_w2, c, w_mod):
        out = pl.pallas_call(
            kernel,
            out_shape=jax.ShapeDtypeStruct((B, D), BF16),
            in_specs=[pl.BlockSpec(memory_space=pltpu.HBM)] * 10,
            out_specs=pl.BlockSpec(memory_space=pltpu.VMEM),
            scratch_shapes=[
                pltpu.VMEM((R, 2, HG, TK, DH), BF16),
                pltpu.VMEM((4, D // 4, H * DH), BF16),
                pltpu.VMEM((4, H * DH // 4, D), BF16),
                pltpu.VMEM((F, D), BF16),
                pltpu.VMEM((F, D), BF16),
                pltpu.VMEM((F, D), BF16),
                pltpu.VMEM((4, D // 4, 6 * D), BF16),
                pltpu.VMEM((2, B, D), BF16),
                pltpu.VMEM((16, D), BF16),
                pltpu.VMEM((16, D), BF16),
                pltpu.VMEM((4, 16, DH), F32),
                pltpu.VMEM((4, 16, DH), F32),
                pltpu.VMEM((16, 4 * D), F32),
                pltpu.VMEM((16, D), F32),
                pltpu.SemaphoreType.DMA((R,)),
                pltpu.SemaphoreType.DMA((NWS,)),
            ],
            compiler_params=pltpu.CompilerParams(
                vmem_limit_bytes=64 * 1024 * 1024,
                disable_bounds_checks=True,
                disable_semaphore_checks=nosem,
            ),
        )(A_x.reshape(B, D), A_k_cache, A_v_cache, A_wq.reshape(4, D // 4, H * DH), A_wo.reshape(4, H * DH // 4, D),
          B_w1.T, B_w3.T, B_w2, c, w_mod.reshape(4, D // 4, 6 * D))
        return out.reshape(B, 1, D)
    return fn


@jax.jit
def pallas_adaLN_cond__sliding_block_cached__glu_gated_swiglu__decode_kernel(
    A_x, A_k_cache, A_v_cache, A_wq, A_wo, B_x, B_w1, B_w3, B_w2, c, w_mod,
):
    return make()(A_x, A_k_cache, A_v_cache, A_wq, A_wo, B_x, B_w1, B_w3, B_w2, c, w_mod)
```

```python
import jax
import jax.numpy as jnp
from jax import lax
import jax.experimental.pallas as pl
import jax.experimental.pallas.tpu as pltpu

F32 = jnp.float32
BF16 = jnp.bfloat16
NT = (((1,), (1,)), ((), ()))

B, H, SK, DH, D, F = 2, 32, 16384, 128, 512, 1376
W = min(4096, max(256, SK // 4))
HG = 8
TK = 128
UPG = W // TK
NG = H // HG
NU = NG * B * UPG
RING = 8
LA = RING - 1
K_DMA = (4, 32)
V_DMA = (2, 64)
FP = -(-F // 128) * 128
FB = 32
NFB = F // FB
CH13 = (0, 512, 1024, F)
CH2 = (0, 512, 896, F)
S_X, S_C, S_M1, S_M2, S_WO, S_Q = range(6)
S_13 = S_Q + NG
S_2 = S_13 + len(CH13) - 1
N_WSEM = S_2 + len(CH2) - 1


def _kernel(x_hbm, k_hbm, v_hbm, wq_hbm, wo_hbm, w1_hbm, w3_hbm, w2_hbm, c_hbm, wm_hbm, o_ref,
            kv, wq, wo, w1, w3, w2, wm, xc, sc_s, h1_s, q_s, o_s, mod_s, at_s, ksem, wsem):
    def mult(v, m):
        return v if isinstance(v, int) else pl.multiple_of(v, m)

    def start(*copies):
        for i, cp in enumerate(copies):
            cp.start(priority=i % 2)

    def wait_filled(dst, sem):
        pltpu.make_async_copy(dst, dst, sem).wait()

    def kv_start(u):
        s = u & (RING - 1)
        b = (u >> 5) & 1
        h0 = (u >> 6) * HG
        r0 = SK - W + (u & (UPG - 1)) * TK
        lists = []
        for j, (src, (nh, nr)) in enumerate(((k_hbm, K_DMA), (v_hbm, V_DMA))):
            lists.append([
                pltpu.make_async_copy(
                    src.at[b, pl.ds(h0 + a * nh, nh), pl.ds(mult(r0 + t * nr, nr), nr)],
                    kv.at[s, j, pl.ds(a * nh, nh), pl.ds(t * nr, nr)], ksem.at[s])
                for t in range(TK // nr) for a in range(HG // nh)])
        start(*[cp for pair in zip(*lists) for cp in pair])

    def kv_wait(u):
        s = u & (RING - 1)
        wait_filled(kv.at[s], ksem.at[s])

    def w_copy(src, dst, si, r, c):
        r, c = mult(r, 8), mult(c, 512)
        return pltpu.make_async_copy(src.at[:, pl.ds(r, 8), pl.ds(c, 512)],
                                     dst.at[:, pl.ds(r, 8), pl.ds(c, 512)], wsem.at[si])

    def w_start(src, dst, si, r, c):
        start(w_copy(src, dst, si, r, c), w_copy(src, dst, si, r, c + 512))

    def w_wait(dst, si, c0, nc):
        wait_filled(dst.at[:, :, pl.ds(mult(c0, 512), nc)], wsem.at[si])

    def f_copy(src, dst, si, edges, j):
        r = mult(j * FB, FB)
        for e in edges[1:-1]:
            si = si + (r >= e).astype(jnp.int32)
        return pltpu.make_async_copy(src.at[pl.ds(r, FB)], dst.at[pl.ds(r, FB)], wsem.at[si])

    def f_start(p0, p1):
        @pl.loop(p0, p1)
        def _(p):
            j = 2 * (p - NFB)

            @pl.when(p < NFB)
            def _():
                start(f_copy(w1_hbm, w1, S_13, CH13, p), f_copy(w3_hbm, w3, S_13, CH13, p))

            @pl.when(p >= NFB)
            def _():
                f_copy(w2_hbm, w2, S_2, CH2, j).start(priority=0)

            @pl.when((p >= NFB) & (j + 1 < NFB))
            def _():
                f_copy(w2_hbm, w2, S_2, CH2, j + 1).start(priority=1)
    n_fpairs = NFB + (NFB + 1) // 2

    def layernorm(x):
        xm = x - jnp.mean(x, axis=-1, keepdims=True)
        return xm / jnp.sqrt(jnp.mean(xm * xm, axis=-1, keepdims=True) + 1e-5)

    def rep8(a):
        return jnp.concatenate([jnp.broadcast_to(a[b:b + 1], (8, a.shape[1])) for b in range(B)], axis=0)

    def mm_slabs(lhs, w, c0):
        c0 = mult(c0, 256)
        return sum(jnp.dot(lhs[:, k * 128:(k + 1) * 128], w[k, :, pl.ds(c0, 256)],
                           preferred_element_type=F32) for k in range(4))

    head8 = lax.broadcasted_iota(jnp.int32, (HG, DH), 0)
    head16 = lax.broadcasted_iota(jnp.int32, (B * HG, DH), 0) & (HG - 1)

    def mod_part(j):
        mod_s[:, pl.ds(mult(j * 256, 256), 256)] = mm_slabs(sc_s[...], wm, j * 256)

    def q_part(g, j):
        qq = mm_slabs(h1_s[...], wq, g * (HG * DH) + j * 256)
        new = jnp.where(head16 == 2 * j, qq[:, :DH], qq[:, DH:])
        q_s[g] = jnp.where((head16 >> 1) == j, new, q_s[g])

    def wo_part(g, j):
        o = o_s[g]
        acc = at_s[...]
        for e in range(2):
            h = 2 * j + e
            lhs = jnp.where(head16 == h, o, 0.0).astype(BF16)
            acc = acc + jnp.dot(lhs, wo[g, pl.ds(mult(h * DH, DH), DH), :], preferred_element_type=F32)
        at_s[...] = acc

    def rows_of(u):
        return u >> 6, pl.ds(mult(((u >> 5) & 1) * HG, HG), HG)

    def scores(u):
        g, rows = rows_of(jnp.minimum(u, NU - 1))
        q = q_s[g, rows, :].astype(BF16)
        s = None
        for h in range(HG):
            r = lax.dot_general(q, kv[u & (RING - 1), 0, h], NT, preferred_element_type=F32)
            s = r if s is None else jnp.where(head8 == h, r, s)
        return s * (DH ** -0.5)

    def softmax_pv(u, s, m, l, acc):
        first = (u & (UPG - 1)) == 0
        m = jnp.where(first, -jnp.inf, m)
        l = jnp.where(first, 0.0, l)
        acc = jnp.where(first, 0.0, acc)
        m_new = jnp.maximum(m, jnp.max(s, axis=-1, keepdims=True))
        alpha = jnp.exp(m - m_new)
        p = jnp.exp(s - m_new)
        pb = p.astype(BF16)
        o = None
        for h in range(HG):
            r = jnp.dot(pb, kv[u & (RING - 1), 1, h], preferred_element_type=F32)
            o = r if o is None else jnp.where(head8 == h, r, o)
        return m_new, alpha * l + p, alpha * acc + o

    cp_c = pltpu.make_async_copy(c_hbm, xc.at[0], wsem.at[S_C])
    cp_x = pltpu.make_async_copy(x_hbm, xc.at[1], wsem.at[S_X])
    start(cp_c, cp_x)
    pl.loop(0, 16)(lambda i: w_start(wm_hbm, wm, S_M1, i * 8, 0))
    pl.loop(0, 16)(lambda i: w_start(wq_hbm, wq, S_Q, i * 8, 0))
    pl.loop(0, LA - 4)(kv_start)
    cp_c.wait()
    cp_x.wait()
    cv = xc[0].astype(F32)
    sc_s[...] = rep8(cv * jax.nn.sigmoid(cv)).astype(BF16)
    ln_x = layernorm(rep8(xc[1].astype(F32)))
    at_s[...] = jnp.zeros(at_s.shape, F32)
    q_s[...] = jnp.zeros(q_s.shape, F32)
    for w in (w1, w3, w2):
        w[F:FP, :] = jnp.zeros((FP - F, D), BF16)

    w_wait(wm, S_M1, 0, 2 * D)

    @pl.loop(0, 4)
    def _(j):
        mod_part(j)
        pl.when((j & 1) == 1)(lambda: kv_start(LA - 4 + (j >> 1)))

    h1_s[...] = (ln_x * (1.0 + mod_s[:, D:2 * D]) + mod_s[:, 0:D]).astype(BF16)
    w_wait(wq, S_Q, 0, HG * DH)

    @pl.loop(0, 4)
    def _(j):
        q_part(0, j)
        pl.when((j & 1) == 1)(lambda: kv_start(LA - 2 + (j >> 1)))

    def side_work(u):
        @pl.when(u < 48)
        def _():
            g = (u >> 4) + 1
            w_start(wq_hbm, wq, S_Q + g, (u & 15) * 8, g * (HG * DH))

        @pl.when((u >= 48) & (u < 80))
        def _():
            w_start(wm_hbm, wm, S_M2, (u & 15) * 8, ((u >> 4) - 2) * 1024)

        @pl.when((u >= 80) & (u < 144))
        def _():
            r = (u - 80) * 8
            start(w_copy(wo_hbm, wo, S_WO, r, 0), w_copy(wo_hbm, wo, S_WO, 512 + r, 0))

        g, v = (u >> 6) + 1, u & 63
        pl.when((v == 56) & (g < NG))(lambda: w_wait(wq, S_Q + g, g * (HG * DH), HG * DH))
        pl.when((v >= 56) & (v < 60) & (g < NG))(lambda: q_part(g, v - 56))
        pl.when(u == 96)(lambda: w_wait(wm, S_M2, 2 * D, 4 * D))
        pl.when((u >= 96) & (u < 104))(lambda: mod_part(u - 92))
        pl.when(u == 160)(lambda: w_wait(wo, S_WO, 0, D))

        @pl.when(((u >= 160) & (u < 168)) | ((u >= 200) & (u < 204)))
        def _():
            i = jnp.where(u < 168, u - 160, u - 192)
            wo_part(i >> 2, i & 3)

    def unit(u, carry):
        s, m, l, acc = carry
        nxt = u + LA
        pl.when(u + 1 < NU)(lambda: kv_wait(u + 1))
        pl.when(nxt < NU)(lambda: kv_start(nxt))
        pl.when(nxt >= NU)(lambda: f_start((nxt - NU) * 8, (nxt - NU + 1) * 8))
        side_work(u)
        s_next = scores(u + 1)
        m, l, acc = softmax_pv(u, s, m, l, acc)

        @pl.when((u & (UPG - 1)) == UPG - 1)
        def _():
            g, rows = rows_of(u)
            o_s[g, rows, :] = acc / jnp.sum(l, axis=-1, keepdims=True)

        return s_next, m, l, acc

    kv_wait(0)
    zero = jnp.zeros((HG, DH), F32)
    lax.fori_loop(0, NU, unit, (scores(0), jnp.full((HG, 1), -jnp.inf, F32), zero, zero))

    p = LA * 8
    per = -(-(n_fpairs - p) // 3)
    for j in range(4):
        wo_part(NG - 1, j)
        if p < n_fpairs:
            f_start(p, min(p + per, n_fpairs))
            p += per

    is0 = lax.broadcasted_iota(jnp.int32, (8, D), 0) == 0
    two = lambda a0, a1: jnp.where(is0, a0, a1)
    mod = lambda j: two(mod_s[0:8, j * D:(j + 1) * D], mod_s[8:16, j * D:(j + 1) * D])
    attn = two(jnp.sum(at_s[0:8], axis=0, keepdims=True), jnp.sum(at_s[8:16], axis=0, keepdims=True))
    x0 = xc[1].astype(F32)
    x1 = two(x0[0:1], x0[1:2]) + mod(2) * attn
    h2 = (layernorm(x1) * (1.0 + mod(4)) + mod(3)).astype(BF16)

    def chunks(edges):
        return [(i, r0, r1 - r0, FP if r1 == F else r1)
                for i, (r0, r1) in enumerate(zip(edges[:-1], edges[1:]))]

    hidden = []
    for i, r0, n, r1 in chunks(CH13):
        wait_filled(w1.at[pl.ds(r0, n)], wsem.at[S_13 + i])
        wait_filled(w3.at[pl.ds(r0, n)], wsem.at[S_13 + i])
        gate = lax.dot_general(h2, w1[r0:r1, :], NT, preferred_element_type=F32)
        up = lax.dot_general(h2, w3[r0:r1, :], NT, preferred_element_type=F32)
        hidden.append((gate * jax.nn.sigmoid(gate) * up).astype(BF16))
    hidden = jnp.concatenate(hidden, axis=1)
    ff = None
    for i, r0, n, r1 in chunks(CH2):
        wait_filled(w2.at[pl.ds(r0, n)], wsem.at[S_2 + i])
        r = jnp.dot(hidden[:, r0:r1], w2[r0:r1, :], preferred_element_type=F32)
        ff = r if ff is None else ff + r
    o_ref[...] = (x1 + mod(5) * ff)[0:B].astype(o_ref.dtype)


@jax.jit
def pallas_adaLN_cond__sliding_block_cached__glu_gated_swiglu__decode_kernel(
    A_x: jax.Array,
    A_k_cache: jax.Array,
    A_v_cache: jax.Array,
    A_wq: jax.Array,
    A_wo: jax.Array,
    B_x: jax.Array,
    B_w1: jax.Array,
    B_w3: jax.Array,
    B_w2: jax.Array,
    c: jax.Array,
    w_mod: jax.Array,
):
    del B_x
    assert A_k_cache.shape == A_v_cache.shape == (B, H, SK, DH)
    out = pl.pallas_call(
        _kernel,
        out_shape=jax.ShapeDtypeStruct((B, D), A_x.dtype),
        in_specs=[pl.BlockSpec(memory_space=pltpu.HBM)] * 10,
        out_specs=pl.BlockSpec(memory_space=pltpu.VMEM),
        scratch_shapes=[
            pltpu.VMEM((RING, 2, HG, TK, DH), BF16),
            pltpu.VMEM((4, D // 4, H * DH), BF16),
            pltpu.VMEM((4, H * DH // 4, D), BF16),
            pltpu.VMEM((FP, D), BF16),
            pltpu.VMEM((FP, D), BF16),
            pltpu.VMEM((FP, D), BF16),
            pltpu.VMEM((4, D // 4, 6 * D), BF16),
            pltpu.VMEM((2, B, D), BF16),
            pltpu.VMEM((B * 8, D), BF16),
            pltpu.VMEM((B * 8, D), BF16),
            pltpu.VMEM((NG, B * HG, DH), F32),
            pltpu.VMEM((NG, B * HG, DH), F32),
            pltpu.VMEM((B * 8, 6 * D), F32),
            pltpu.VMEM((B * 8, D), F32),
            pltpu.SemaphoreType.DMA((RING,)),
            pltpu.SemaphoreType.DMA((N_WSEM,)),
        ],
        compiler_params=pltpu.CompilerParams(
            vmem_limit_bytes=48 * 1024 * 1024,
            disable_bounds_checks=True,
            disable_semaphore_checks=True,
        ),
    )(A_x.reshape(B, D), A_k_cache, A_v_cache,
      A_wq.reshape(4, D // 4, H * DH), A_wo.reshape(4, H * DH // 4, D),
      B_w1.T, B_w3.T, B_w2, c, w_mod.reshape(4, D // 4, 6 * D))
    return out.reshape(B, 1, D)
```
